```python
import os as _os
_os.environ.setdefault('JAX_PLATFORMS', 'cpu')
import jax
import jax.numpy as jnp

def _softmax(x, axis=-1):
    return jax.nn.softmax(x, axis=axis)

def _gelu(x):
    return jax.nn.gelu(x, approximate=True)

def _silu(x):
    return jax.nn.silu(x)

def _sigmoid(x):
    return jax.nn.sigmoid(x)

def _layernorm(x, axis=-1, eps=1e-05):
    m = jnp.mean(x, axis=axis, keepdims=True)
    v = jnp.var(x, axis=axis, keepdims=True)
    return (x - m) / jnp.sqrt(v + eps)

def _scatter_add(tgt, idx, src, axis=0):
    return tgt.at[idx].add(src)

def _segment_sum(src, seg, n):
    return jax.ops.segment_sum(src, seg, n)

class _Rng:

    def __init__(self, key):
        self._k = key

    def _next(self):
        self._k, sub = jax.random.split(self._k)
        return sub

    def normal(self, shape):
        return jax.random.normal(self._next(), shape, dtype=jnp.bfloat16)

    def randint(self, lo, hi, shape):
        return jax.random.randint(self._next(), shape, lo, hi, dtype=jnp.int32)

    def uniform(self, shape, lo=0.0, hi=1.0):
        return jax.random.uniform(self._next(), shape, jnp.bfloat16, lo, hi)

    def permutation(self, n):
        return jax.random.permutation(self._next(), n)
kernel_name = 'adaLN_cond__sliding_block__mixer_channel_mlp__prompt'

def setup_inputs():
    _rng = _Rng(jax.random.key(int.from_bytes(__import__("os").urandom(4), "little")))
    _w = lambda a: (lambda t: t.astype(jnp.bfloat16) if jnp.issubdtype(t.dtype, jnp.floating) else t)(jnp.asarray(a))

    def _A_setup():
        B, S, D = (1, 2048, 640)
        return {'x': _w((lambda *s: _rng.normal(s) * 0.05)(B, S, D)), 'wqkv': _w((lambda *s: _rng.normal(s) * 0.05)(D, 3 * D)), 'wo': _w((lambda *s: _rng.normal(s) * 0.05)(D, D))}
    _A_in = _A_setup()

    def _B_setup():
        B, S, D, F = (1, 2048, 640, 1728)
        return {'x': _w((lambda *s: _rng.normal(s) * 0.05)(B, S, D)), 'w1': _w((lambda *s: _rng.normal(s) * 0.8)(D, F) * D ** (-0.5)), 'b1': _w((lambda *s: _rng.normal(s) * 0.8)(F)), 'w2': _w((lambda *s: _rng.normal(s) * 0.8)(F, D) * F ** (-0.5)), 'b2': _w((lambda *s: _rng.normal(s) * 0.4)(D))}
    _B_in = _B_setup()
    return {'A_x': _A_in['x'], 'A_wqkv': _A_in['wqkv'], 'A_wo': _A_in['wo'], 'B_x': _B_in['x'], 'B_w1': _B_in['w1'], 'B_b1': _B_in['b1'], 'B_w2': _B_in['w2'], 'B_b2': _B_in['b2'], 'c': _w((lambda *s: _rng.normal(s) * 0.05)(1, 640) * 8.0), 'w_mod': _w((lambda *s: _rng.normal(s) * 0.05)(640, 6 * 640) * 640 ** (-0.5) * 8.0)}

def reference(A_x, A_wqkv, A_wo, B_x, B_w1, B_b1, B_w2, B_b2, c, w_mod):

    def _A_ref(x, wqkv, wo):
        B, S, D = x.shape
        H = 32
        Dh = D // H
        W = 256
        qkv = (lambda x, *d: x.transpose(*d))((x @ wqkv).reshape(B, S, 3, H, Dh), 2, 0, 3, 1, 4)
        q, k, v = (qkv[0], qkv[1], qkv[2])
        scores = jnp.einsum('bhqd,bhkd->bhqk', q, k) * Dh ** (-0.5)
        idx = jnp.arange(S)
        mask = (idx[:, None] - idx[None, :] >= 0) & (idx[:, None] - idx[None, :] < W)
        scores = jnp.where(mask[None, None], scores, -1000000000.0)
        p = _softmax(scores, axis=-1)
        o = jnp.einsum('bhqk,bhkd->bhqd', p, v)
        return (lambda x, *d: x.transpose(*d))(o, 0, 2, 1, 3).reshape(B, S, D) @ wo

    def _B_ref(x, w1, b1, w2, b2):
        y = _layernorm(x, axis=-1)
        h = _gelu(jnp.einsum('bsd,df->bsf', y, w1) + b1)
        return jnp.einsum('bsf,fd->bsd', h, w2) + b2
    x = A_x
    mod = (_silu(c) @ w_mod).reshape(c.shape[0], 6, 1, -1)
    sa, ca, ga, sb, cb, gb = (mod[:, 0].copy(), mod[:, 1].copy(), mod[:, 2].copy(), mod[:, 3].copy(), mod[:, 4].copy(), mod[:, 5].copy())
    h = _layernorm(x, axis=-1) * (1 + ca) + sa
    x = x + ga * _A_ref(h, A_wqkv, A_wo)
    h = _layernorm(x, axis=-1) * (1 + cb) + sb
    x = x + gb * _B_ref(h, B_w1, B_b1, B_w2, B_b2)
    return x
```

```python
import functools
import math
import jax
import jax.numpy as jnp
from jax import lax
import jax.experimental.pallas as pl
import jax.experimental.pallas.tpu as pltpu

S, D, F, H, DH, W = 2048, 640, 1728, 32, 20, 256
TQ = 256
DMAMODE = 0
NQB = TQ // 128
NG = 8
EPS = 1e-5
QSCALE = (DH ** -0.5) * math.log2(math.e)
NEG = -1e30
f32, bf16, u32 = jnp.float32, jnp.bfloat16, jnp.uint32

NT = (((1,), (1,)), ((), ()))


def _ln(x):
    m = jnp.mean(x, axis=-1, keepdims=True)
    xc = x - m
    v = jnp.mean(xc * xc, axis=-1, keepdims=True)
    return xc * lax.rsqrt(v + EPS)


def _gelu(x):
    c = math.sqrt(2.0 / math.pi)
    u = x * (c + (c * 0.044715) * (x * x))
    hx = 0.5 * x
    return hx + hx * jnp.tanh(u)


def _to32(x):
    return pltpu.bitcast(x, u32)


def _to16(x):
    return pltpu.bitcast(x, bf16)


def _circ_mask(lane, start, size):
    start %= 128
    end = start + size
    if end <= 128:
        return (lane >= start) & (lane < end)
    return (lane >= start) | (lane < end - 128)


def _colmax8(blocks):
    acc = [None, None]
    n = 0
    for blk in blocks:
        for r in range(0, blk.shape[0], 8):
            v = blk[r:r + 8]
            acc[n % 2] = v if acc[n % 2] is None else jnp.maximum(acc[n % 2], v)
            n += 1
    return jnp.maximum(acc[0], acc[1])


def kernel(x_ref, wqkv_hbm, wo_hbm, w1t_hbm, b1_ref, w2_hbm, b2_ref, c_ref, wmod_hbm,
           o_ref,
           wqkv_ref, wo_ref, w1t_ref, w2_ref, wmod_ref, sems,
           mod_ref, bias_ref, wvt_ref, q_ref, k_ref, vt_ref):
    step = pl.program_id(0)

    def cp(src, dst, lo, hi, i):
        src = src.bitcast(u32)
        if lo is not None:
            src, dst = src.at[:, lo:hi], dst.at[:, lo:hi]
        return pltpu.make_async_copy(src, dst, sems.at[i])

    cps = dict(
        ma=cp(wmod_hbm, wmod_ref, 0, 2 * D, 0),
        qk=cp(wqkv_hbm, wqkv_ref, 0, 2 * D, 1),
        v=cp(wqkv_hbm, wqkv_ref, 2 * D, 3 * D, 2),
        o=cp(wo_hbm, wo_ref, None, None, 3),
        mb=cp(wmod_hbm, wmod_ref, 2 * D, 5 * D, 4),
        w1=cp(w1t_hbm, w1t_ref, None, None, 5),
        w2=cp(w2_hbm, w2_ref, None, None, 6),
        mc=cp(wmod_hbm, wmod_ref, 5 * D, 6 * D, 7),
    )

    def body(first):
        lane64 = lax.broadcasted_iota(jnp.int32, (64, 128), 1)
        lane16 = lax.broadcasted_iota(jnp.int32, (16, 128), 1)
        row32 = lax.broadcasted_iota(jnp.int32, (32, 128), 0)
        lane32 = lax.broadcasted_iota(jnp.int32, (32, 128), 1)
        bit0 = (lane32 & 32) == 0
        bit1 = (lane32 & 64) == 0
        mask_up = row32 > (lane32 & 31)
        sub8 = lax.broadcasted_iota(jnp.int32, (8, 128), 0) < 4
        zero16 = jnp.zeros((16, 128), u32)
        neg32 = jnp.full((32, 128), NEG, f32)
        lane640 = lax.broadcasted_iota(jnp.int32, (32, D), 1)
        hcls = lane640 // DH
        obit0 = (hcls & 1) == 0
        obit1 = (hcls & 2) == 0
        ones8 = jnp.ones((8, 128), f32)
        row128 = lax.broadcasted_iota(jnp.int32, (128, 128), 0)
        lane128 = lax.broadcasted_iota(jnp.int32, (128, 128), 1)
        st = {}
        waited = set()

        def modv(i):
            return mod_ref[0:1, i * D:(i + 1) * D]

        def need(name):
            if not first or name in waited:
                return
            waited.add(name)
            cps[name].wait()
            if DMAMODE == 1:
                nxt = dict(ma=("v", "o"), qk=("mb", "w1"), v=("w2", "mc")).get(name, ())
                for nm in nxt:
                    cps[nm].start()
            if name in ("ma", "mb", "mc"):
                lo, hi = dict(ma=(0, 2), mb=(2, 5), mc=(5, 6))[name]
                r = jnp.dot(st["sc"], _to16(wmod_ref[:, lo * D:hi * D]),
                            preferred_element_type=f32)[0:8]
                if name == "ma":
                    r = r + jnp.where(lax.broadcasted_iota(jnp.int32, r.shape, 1) >= D, 1.0, 0.0)
                if name == "mb":
                    r = r + jnp.where(lax.broadcasted_iota(jnp.int32, r.shape, 1) >= 2 * D, 1.0, 0.0)
                mod_ref[:, lo * D:hi * D] = r
            if name == "v":
                wvt_ref[...] = _to32(_to16(wqkv_ref[:, 2 * D:3 * D]).T)

        if first:
            names = ("ma", "qk") if DMAMODE == 1 else ("ma", "qk", "v", "o", "mb", "w1", "w2", "mc")
            for nm in names:
                cps[nm].start()
            c = c_ref[...].astype(f32)
            sc = c * jax.nn.sigmoid(c)
            st["sc"] = jnp.broadcast_to(sc, (16, D)).astype(bf16)
            bias_ref[0:1, 0:F] = b1_ref[...].astype(f32).reshape(1, F)
            bias_ref[1:2, 0:D] = b2_ref[...].astype(f32).reshape(1, D)

        def ln1(b):
            x = x_ref[128 * b:128 * b + 128, :].astype(f32)
            n = _ln(x)
            need("ma")
            st["h", b] = (n * modv(1) + modv(0)).astype(bf16)

        def qproj(b):
            need("qk")
            q = jnp.dot(st["h", b], _to16(wqkv_ref[:, 0:D]), preferred_element_type=f32)
            q_ref[64 * b:64 * b + 64, :] = _to32((q * QSCALE).astype(bf16))

        def kproj(b):
            need("qk")
            k = jnp.dot(st["h", b], _to16(wqkv_ref[:, D:2 * D]), preferred_element_type=f32)
            kp = _to32(k.astype(bf16))
            for g in range(NG):
                start = (80 * g) % 128
                a = (80 * g) // 128
                ka = kp[:, 128 * a:128 * a + 128]
                if start + 80 > 128:
                    ka = jnp.where(lane64 >= start, ka, kp[:, 128 * a + 128:128 * a + 256])
                k_ref[W // 2 + 64 * b:W // 2 + 64 * b + 64, 128 * g:128 * g + 128] = ka

        def vproj(b):
            need("v")
            vt = lax.dot_general(_to16(wvt_ref[...]), st.pop(("h", b)), NT,
                                 preferred_element_type=f32)
            pieces = []
            for p in range(H // 2):
                pieces += [vt[40 * p:40 * p + 24], ones8, vt[40 * p + 24:40 * p + 40]]
            vt_ref[:, W + 128 * b:W + 128 * b + 128] = _to32(
                jnp.concatenate(pieces, axis=0).astype(bf16))

        def kt0(b):
            return max(0, 2 - b) if first else 0

        def sel(m, a, b):
            if a is None and b is None:
                return None
            return jnp.where(m, neg32 if a is None else a, neg32 if b is None else b)

        def stage_a(b, g):
            start = (80 * g) % 128
            a = (80 * g) // 128
            cols = slice(128 * g, 128 * g + 128)
            hm = [_circ_mask(lane16, start + DH * i, DH) for i in range(4)]
            qs = []
            for j in range(4):
                r = slice(64 * b + 16 * j, 64 * b + 16 * j + 16)
                qj = q_ref[r, 128 * a:128 * a + 128]
                if start + 80 > 128:
                    qj = jnp.where(lane16 >= start, qj, q_ref[r, 128 * a + 128:128 * a + 256])
                qs.append(qj)
            t0 = 64 * b
            t2 = t0 + 128
            u = []
            for j in range(4):
                qm = jnp.concatenate([jnp.where(hm[c ^ j], qs[j], zero16) for c in range(4)], axis=0)
                kw = k_ref[t2:t2 + 16 * (j + 1), cols]
                if kt0(b) == 0:
                    kw = jnp.concatenate([kw, k_ref[t0 + 16 * j:t0 + 64, cols]], axis=0)
                s = lax.dot_general(_to16(kw), _to16(qm), NT, preferred_element_type=f32)
                blk = [s[32 * r:32 * r + 32] for r in range(s.shape[0] // 32)]
                if kt0(b) == 0:
                    u.append(blk[:j] + [jnp.where(mask_up, blk[j + 1], blk[j])] + blk[j + 2:])
                else:
                    u.append(blk[:j] + [jnp.where(mask_up, NEG, blk[j])] + [None] * (3 - j))
            if kt0(b) <= 1:
                qm = jnp.concatenate([jnp.where(hm[i], qs[c ^ i], zero16)
                                      for i in range(4) for c in range(4)], axis=0)
                smid = lax.dot_general(_to16(k_ref[t0 + 64:t0 + 128, cols]), _to16(qm), NT,
                                       preferred_element_type=f32)
            e = [[], [], [], []]
            for r in range(4):
                t = [sel(bit0, u[j][r], u[j ^ 1][r]) for j in range(4)]
                for i in range(4):
                    e[i].append(sel(bit1, t[i], t[i ^ 2]))
            res = []
            for i in range(4):
                se = jnp.concatenate(e[i], axis=0)
                sm = smid[:, 128 * i:128 * i + 128] if kt0(b) <= 1 else None
                m8 = _colmax8([se] + ([sm] if sm is not None else []))
                m = jnp.max(m8, axis=0, keepdims=True)
                res.append((se, sm, m))
            st["s", b, g] = res

        def stage_c(b, g):
            res = [None] * 4
            tiles = [[], [], []]
            for i, (se, sm, m) in enumerate(st.pop(("s", b, g))):
                pe = jnp.exp2(se - m)
                if sm is not None:
                    tiles[1].append(jnp.exp2(sm - m).astype(bf16))
                if kt0(b) == 0:
                    up = row128 > (lane128 ^ (32 * i))
                    tiles[0].append(jnp.where(up, pe, 0.0).astype(bf16))
                    tiles[2].append(jnp.where(up, 0.0, pe).astype(bf16))
                else:
                    tiles[2].append(pe.astype(bf16))
            for kt in (1, 0, 2):
                for i, pi in enumerate(tiles[kt]):
                    hd = 4 * g + i
                    ro = 24 * (hd // 2) + 8 * (hd % 2)
                    c0 = 128 * (b + kt)
                    vw = _to16(vt_ref[ro:ro + 16, c0:c0 + 128])
                    d = jnp.dot(vw, pi, preferred_element_type=f32)
                    res[i] = d if res[i] is None else res[i] + d
            rows = []
            for e in (0, 2):
                re, rod = res[e], res[e + 1]
                ie = 1.0 / re[24:32]
                io = 1.0 / rod[8:16]
                rows += [re[0:8] * ie, re[8:16] * ie,
                         jnp.where(sub8, re[16:24] * ie, rod[0:8] * io),
                         rod[16:24] * io, rod[24:32] * io]
            st.setdefault(("ot", b), []).extend(rows)

        def oproj(b):
            ot = jnp.concatenate(st.pop(("ot", b)), axis=0)
            op = ot.T
            blk = [op[32 * c:32 * c + 32] for c in range(4)]
            t = [jnp.where(obit0, blk[j], blk[j ^ 1]) for j in range(4)]
            o = jnp.concatenate([jnp.where(obit1, t[j], t[j ^ 2]) for j in range(4)],
                                axis=0).astype(bf16)
            need("o")
            need("mb")
            attn = jnp.dot(o, _to16(wo_ref[...]), preferred_element_type=f32)
            x1 = x_ref[128 * b:128 * b + 128, :].astype(f32) + modv(2) * attn
            h2 = _ln(x1) * modv(4) + modv(3)
            st["y", b] = _ln(h2).astype(bf16)
            st["x1", b] = x1

        def mlp1(b, lo, hi):
            need("w1")
            h1 = lax.dot_general(st["y", b], _to16(w1t_ref[lo // 2:hi // 2, :]), NT,
                                 preferred_element_type=f32)
            h1 = h1 + bias_ref[0:1, lo:hi]
            st.setdefault(("g1", b), []).append(_gelu(h1))

        def mlp2(b, lo, hi):
            need("w2")
            need("mc")
            if isinstance(st["g1", b], list):
                st["g1", b] = jnp.concatenate(st["g1", b], axis=1).astype(bf16)
            out = jnp.dot(st["g1", b], _to16(w2_ref[:, lo:hi]), preferred_element_type=f32)
            out = out + bias_ref[1:2, lo:hi]
            o_ref[128 * b:128 * b + 128, lo:hi] = (
                st["x1", b][:, lo:hi] + mod_ref[0:1, 5 * D + lo:5 * D + hi] * out).astype(o_ref.dtype)

        def front_tasks(b):
            return [(0, functools.partial(ln1, b)),
                    (800, functools.partial(kproj, b)),
                    (800, functools.partial(qproj, b)),
                    (800, functools.partial(vproj, b))]

        def w1_tasks(b):
            edges = [0, 512, 1024, 1408, F]
            return [(160 * -(-(hi - lo) // 128), functools.partial(mlp1, b, lo, hi))
                    for lo, hi in zip(edges[:-1], edges[1:])]

        def w2_tasks(b):
            return [(448, functools.partial(mlp2, b, 128 * n, 128 * n + 128)) for n in range(5)]

        def slide():
            k_ref[0:W // 2, :] = k_ref[TQ // 2:TQ // 2 + W // 2, :]
            vt_ref[:, 0:W] = vt_ref[:, TQ:TQ + W]

        for _, t in front_tasks(0):
            t()
        carry = []
        for b in range(NQB):
            fill = list(carry)
            carry = []
            fr = front_tasks(b + 1) if b + 1 < NQB else []
            if b > 0:
                fill += [(800, functools.partial(oproj, b - 1))]
                fill += fr
                if not fr:
                    fill += [(0, None), (0, None)]
                fill += w1_tasks(b - 1)
                w2 = w2_tasks(b - 1)
                if b == NQB - 1:
                    fill += w2[:1]
                    carry = w2[1:]
                else:
                    fill += w2
            else:
                fill += fr
            total = sum(c for c, _ in fill)
            done = 0
            if b == 0:
                stage_a(b, 0)
            for g in range(NG):
                if g + 1 < NG:
                    stage_a(b, g + 1)
                while fill and (done < total * (g + 1) / NG or g == NG - 1):
                    c, t = fill.pop(0)
                    done += c
                    if t is None:
                        break
                    t()
                if g + 1 == NG and b + 1 < NQB:
                    stage_a(b + 1, 0)
                stage_c(b, g)
        slide()
        b = NQB - 1
        carry.pop(0)[1]()
        oproj(b)
        for _, t in carry:
            t()
        for _, t in w1_tasks(b) + w2_tasks(b):
            t()

    pl.when(step == 0)(functools.partial(body, True))
    pl.when(step > 0)(functools.partial(body, False))


@jax.jit
def pallas_adaLN_cond__sliding_block__mixer_channel_mlp__prompt_kernel(A_x, A_wqkv, A_wo, B_x, B_w1, B_b1, B_w2, B_b2, c, w_mod):
    x = A_x.reshape(S, D)
    hbm = pl.BlockSpec(memory_space=pl.ANY)
    out = pl.pallas_call(
        kernel,
        grid=(S // TQ,),
        in_specs=[
            pl.BlockSpec((TQ, D), lambda i: (i, 0)),
            hbm, hbm, hbm,
            pl.BlockSpec((F,), lambda i: (0,)),
            hbm,
            pl.BlockSpec((D,), lambda i: (0,)),
            pl.BlockSpec((1, D), lambda i: (0, 0)),
            hbm,
        ],
        out_specs=pl.BlockSpec((TQ, D), lambda i: (i, 0)),
        out_shape=jax.ShapeDtypeStruct((S, D), A_x.dtype),
        scratch_shapes=[
            pltpu.VMEM((D // 2, 3 * D), u32),
            pltpu.VMEM((D // 2, D), u32),
            pltpu.VMEM((F // 2, D), u32),
            pltpu.VMEM((F // 2, D), u32),
            pltpu.VMEM((D // 2, 6 * D), u32),
            pltpu.SemaphoreType.DMA((8,)),
            pltpu.VMEM((8, 6 * D), f32),
            pltpu.VMEM((8, 1792), f32),
            pltpu.VMEM((D // 2, D), u32),
            pltpu.VMEM((TQ // 2, D), u32),
            pltpu.VMEM(((W + TQ) // 2, NG * 128), u32),
            pltpu.VMEM((24 * 16, W + TQ), u32),
        ],
        compiler_params=pltpu.CompilerParams(
            dimension_semantics=("arbitrary",),
            vmem_limit_bytes=100 * 1024 * 1024),
        name="fused_block",
    )(x, A_wqkv, A_wo, B_w1.T, B_b1, B_w2, B_b2, c, w_mod)
    return out.reshape(1, S, D)
```

```python
import functools
import itertools
import math

import jax
import jax.numpy as jnp
from jax import lax
import jax.experimental.pallas as pl
import jax.experimental.pallas.tpu as pltpu

S, D, F, H, DH, W = 2048, 640, 1728, 32, 20, 256
TQ = 256
FM = 1664
KB = D + 384
NB = S // TQ
NG = 8
LEAD = 2
EPS = 1e-5
QSCALE = (DH ** -0.5) * math.log2(math.e)
NEG = -1e30

FIRST_PRE = (
    "+c,b1,b2,ca,x0,ka ?c,b1,b2,ca +kb,x1 ?x0 +q,sa,v !l0 !l1 !c0 !c1 ?ka +mb,o,w1 @i0*3 "
    "@i1*3 #LLLLLLL ?kb,x1 !l2 !l3 !c2 !c3 @i0*2 @i1*2 @i2*5 @i3*5 #LLLLLLLLLLLLLLLL ?q "
    "+gb,w2 @j0*5 @j1*5 @j2*5 @j3*5 #LLLLLLLLLLLLLLLLLLLLL ?sa,v @m1*5 @v0*5 @v1*5 @v2*5 "
    "@v3*5 @o0*5 @o1*5 #LsssLssLs @b1*5 @b0*5 #sLssLsLsLsLsLLsL !k1 #sLs !k0 #LsLsLLss !q0")
FIRST_FILL = (
    "!q1 #L||#L||!k2 !q2|#LL|#L||#L||!k3 !q3 #L||#L||#L|#L|#L||#L|#L||||||"
    "#L ?mb,o,w1 #L +xb @m0*15 !s0 !s1 #ssssLssL|#sLssLssLsL|#sL|#sLsLsssL|#sL !f0 #L||"
    "#L @u0*13 @u1*13 #L")
FIRST_POST = (
    "#LL !f1 #LLLLLLLL ?gb,w2 @m0*5 #LLsLsLLsLLLLsLsLsLLLsLLLLLLLL t0*2 !s2 !s3 d0*5 d1*5 "
    "?xb")
STEADY_PRE = "!l2 !l3 O0*5 Q2*5 K2*5 v2*4 t0*1 v3*4 t0*1"
STEADY_FILL = ("v2*1 v3*1 u0*2|u0*4|u0*4|u0*3 u1*1|u1*4|u1*4|u1*4|D0*1|"
               "D0*1|!s2 D0*1|D0*1|D0*1|D1*1|D1*1|D1*1|D1*1")
STEADY_POST = "!s3 D1*1"
LAST = "o0*5 o1*5 u0*13 u1*1 t0*2 u1*12 d0*5 d1*3 d1*1 d1*1"

f32, bf16, u32 = jnp.float32, jnp.bfloat16, jnp.uint32
NN = (((1,), (0,)), ((), ()))
NT = (((1,), (1,)), ((), ()))
P = functools.partial


def _ln(x):
    m = jnp.sum(x, axis=-1, keepdims=True) * (1.0 / D)
    xc = x - m
    v = jnp.sum(xc * xc, axis=-1, keepdims=True) * (1.0 / D)
    return xc * jnp.exp2(jnp.log(v + EPS) * (-0.5 * math.log2(math.e)))


def _gelu(x):
    c = math.sqrt(2.0 / math.pi)
    u = x * (c + (c * 0.044715) * (x * x))
    hx = 0.5 * x
    return hx + hx * jnp.tanh(u)


def _to32(x):
    return pltpu.bitcast(x, u32)


def _to16(x):
    return pltpu.bitcast(x, bf16)


def _rows(v8, n):
    return jnp.concatenate([v8] * (n // 8), axis=0)


def _t(k):
    return slice(128 * k, 128 * k + 128)


def _circ_mask(lane, start, size):
    start %= 128
    end = start + size
    if end <= 128:
        return (lane >= start) & (lane < end)
    return (lane >= start) | (lane < end - 128)


def _colmax8(blocks):
    acc = [None, None]
    n = 0
    for blk in blocks:
        for r in range(0, blk.shape[0], 8):
            v = blk[r:r + 8]
            acc[n % 2] = v if acc[n % 2] is None else jnp.maximum(acc[n % 2], v)
            n += 1
    return jnp.maximum(acc[0], acc[1])


def _kernel(x_hbm, wqkv_hbm, wo_hbm, w1t_hbm, b1_hbm, w2_hbm, b2_hbm, c_hbm, wmod_hbm,
            o_hbm,
            o_ref, x_ref, wqkv_in, wo_in, w1t_in, w2_in, wmod_in, b1_ref, b2_ref, c_ref,
            wqk_ref, wo_ref, w1t_ref, w2_ref,
            sems,
            mod_ref, bias_ref, wvt_ref, q_ref, k_ref, vt_ref, a_ref, s_ref, ot_ref, x1_ref,
            hs_ref, raw_ref):
    step = pl.program_id(0)

    def copy(src, dst, lo, hi, i):
        if lo is not None:
            src, dst = src.at[:, lo:hi], dst.at[:, lo:hi]
        return pltpu.make_async_copy(src, dst, sems.at[i])

    cps = dict(
        c=P(copy, c_hbm, c_ref, None, None, 0),
        b1=P(copy, b1_hbm, b1_ref, None, None, 0),
        b2=P(copy, b2_hbm, b2_ref, None, None, 0),
        ca=P(copy, wmod_hbm, wmod_in, D, 2 * D, 0),
        x0=P(copy, x_hbm.at[0:TQ, :], x_ref.at[0:TQ, :], None, None, 1),
        ka=P(copy, wqkv_hbm, wqkv_in, D, KB, 2),
        kb=P(copy, wqkv_hbm, wqkv_in, KB, 2 * D, 0),
        x1=P(copy, x_hbm.at[TQ:2 * TQ, :], x_ref.at[TQ:2 * TQ, :], None, None, 0),
        q=P(copy, wqkv_hbm, wqkv_in, 0, D, 3),
        sa=P(copy, wmod_hbm, wmod_in, 0, D, 1),
        v=P(copy, wqkv_hbm, wqkv_in, 2 * D, 3 * D, 1),
        mb=P(copy, wmod_hbm, wmod_in, 2 * D, 5 * D, 2),
        o=P(copy, wo_hbm, wo_in, None, None, 2),
        w1=P(copy, w1t_hbm, w1t_in, None, None, 2),
        gb=P(copy, wmod_hbm, wmod_in, 5 * D, 6 * D, 3),
        w2=P(copy, w2_hbm, w2_in, None, None, 3),
        xb=P(copy, x_hbm.at[2 * TQ:S, :], x_ref.at[2 * TQ:S, :], None, None, 0),
    )
    osem = sems.at[1]

    def body(mode):
        first = mode == "first"
        row32 = lax.broadcasted_iota(jnp.int32, (32, 128), 0)
        lane32 = lax.broadcasted_iota(jnp.int32, (32, 128), 1)
        bit0 = (lane32 & 32) == 0
        bit1 = (lane32 & 64) == 0
        mask_up = row32 > (lane32 & 31)
        sub8 = lax.broadcasted_iota(jnp.int32, (8, 128), 0) < 4
        neg32 = jnp.full((32, 128), NEG, f32)
        row128 = lax.broadcasted_iota(jnp.int32, (128, 128), 0)
        lane128 = lax.broadcasted_iota(jnp.int32, (128, 128), 1)
        st = {}
        have = set()

        flying = set()

        def chk(*key):
            assert key in have or (not first and (key[0] in "mw" or key[1] < 2)), key

        def memo(key, fn):
            if key not in st:
                st[key] = fn()
            return st[key]

        fblk = 0 if first else step
        bblk = dict(first=0, steady=step, last=NB - 1)[mode]

        def rows(blk, off, n, align=128):
            if isinstance(blk, int):
                return pl.ds(blk * TQ + off, n)
            return pl.ds(pl.multiple_of(blk * TQ + off, align), n)

        if not first:
            r = rows(bblk - 1, 0, TQ)
            pltpu.make_async_copy(o_ref.at[r, :], o_hbm.at[r, :], osem).start()

        def mod(lo, hi, n):
            for t in range(lo // 128, hi // 128):
                chk("m", t)
            return _rows(mod_ref[:, lo:hi], n)

        def modv(i):
            return mod(i * D, (i + 1) * D, 128)

        def weight(name, src, packed, lo, hi, axis):
            chk("w", name)
            pieces = []
            for t in range(lo, hi, 128):
                e = min(hi, t + 128)
                pidx = (slice(None), slice(t, e)) if axis else (slice(t // 2, e // 2), slice(None))
                if first and (name, t) not in st:
                    st[name, t] = True
                    piece = _to32(src[:, t:e] if axis else src[t:e, :])
                    packed[pidx] = piece
                else:
                    piece = packed[pidx]
                pieces.append(piece)
            return jnp.concatenate(pieces, axis=axis)

        def wqk_name(col):
            return "q" if col < D else "ka" if col < KB else "kb"

        def wqk(lo, hi):
            return weight(wqk_name(hi - 1), wqkv_in, wqk_ref, lo, hi, 1)

        wo = P(weight, "o", wo_in, wo_ref, axis=1)
        w1t = P(weight, "w1", w1t_in, w1t_ref, axis=0)
        w2 = P(weight, "w2", w2_in, w2_ref, axis=1)

        def mod_store(lo, r):
            col = lax.broadcasted_iota(jnp.int32, r.shape, 1) + lo
            plus1 = ((col >= D) & (col < 2 * D)) | ((col >= 4 * D) & (col < 5 * D))
            mod_ref[:, lo:lo + r.shape[1]] = r + jnp.where(plus1, 1.0, 0.0)
            have.update(("m", n) for n in range(lo // 128, (lo + r.shape[1]) // 128))

        def wait(names):
            used = {cps[n].args[-1] for n in names}
            assert {n for n in flying if cps[n].args[-1] in used} == set(names)
            flying.difference_update(names)
            have.update(("w", n) for n in names)
            for name in names:
                cps[name]().wait()
            for name in names:
                if name == "c":
                    c = c_ref[...].astype(f32)
                    st["sc"] = jnp.broadcast_to(c * jax.nn.sigmoid(c), (8, D))
                if name == "ca":
                    mod_store(D, jnp.dot(st["sc"], wmod_in[:, D:2 * D], preferred_element_type=f32))
                if name == "v":
                    wvt_ref[...] = _to32(wqkv_in[:, 2 * D:3 * D].T)
                if name == "b1":
                    b1 = jnp.broadcast_to(b1_ref[...].astype(f32).reshape(1, F), (8, F))
                    bias_ref[0:8, 0:F] = b1
                    bias_ref[0:8, F:F + 64] = b1[:, FM:F]
                if name == "b2":
                    bias_ref[8:16, 0:D] = jnp.broadcast_to(
                        b2_ref[...].astype(f32).reshape(1, D), (8, D))

        def ln1(w):
            chk("w", "x%d" % (w // 2))
            st["n", w] = _ln(x_ref[rows(fblk, 128 * w, 128), :].astype(f32))

        def hscale(w):
            hs = st.pop(("n", w)) * modv(1)
            hs_ref[_t(w), :] = hs
            for k in range(5):
                st["hs", w, k] = hs[:, _t(k)].astype(bf16)

        def hmod(w):
            if first:
                assert ("hs", w, 0) in st
                return memo(("hf", w), lambda: hs_ref[_t(w), :] + modv(0))
            return memo(("hf", w), lambda: st.pop(("n", w)) * modv(1) + modv(0))

        def hval(w, nb):
            return memo(("h", w, nb), lambda: jnp.concatenate(
                [hmod(w + i) for i in range(nb)], axis=0).astype(bf16))

        def htile(w, k):
            return memo(("ht", w, k), lambda: hmod(w)[:, _t(k)].astype(bf16))

        def qstore(w, nb, q):
            q_ref[128 * w:128 * (w + nb), :] = q * QSCALE
            have.update(("q", w + i) for i in range(nb))

        def kstore(w, nb, k):
            kp = _to32(k.astype(bf16))
            lane = lax.broadcasted_iota(jnp.int32, (64 * nb, 128), 1)
            for g in range(NG):
                start, a = (80 * g) % 128, (80 * g) // 128
                ka = kp[:, _t(a)]
                if start + 80 > 128:
                    ka = jnp.where(lane >= start, ka, kp[:, _t(a + 1)])
                k_ref[64 * w:64 * (w + nb), _t(g)] = ka
            have.update(("k", w + i) for i in range(nb))

        def vstore(w, r0, r1, vt):
            have.update(("v", w, v) for v in range(r0 // 8, r1 // 8))
            pieces = []
            for v in range(r0 // 8, r1 // 8):
                sl = vt[8 * v - r0:8 * v - r0 + 8]
                if v % 5 == 2:
                    pieces += [jnp.where(sub8, sl, 1.0), jnp.where(sub8, 1.0, sl)]
                else:
                    pieces.append(sl)
            d0 = r0 + 8 * ((r0 // 8 + 2) // 5)
            vt_ref[d0:d0 + 8 * len(pieces), _t(w)] = jnp.concatenate(pieces, axis=0)

        def qproj2(w, n0, n1):
            assert (n0, n1) == (0, 5)
            wq = wqk(0, D)
            qstore(w, 2, jnp.dot(hval(w, 2), _to16(wq), preferred_element_type=f32))

        def kproj2(w, n0, n1):
            assert (n0, n1) == (0, 5)
            wk = wqk(D, 2 * D)
            kstore(w, 2, jnp.dot(hval(w, 2), _to16(wk), preferred_element_type=f32))

        def vproj(w, n0, n1):
            r0, r1 = 128 * n0, 128 * n1
            vstore(w, r0, r1, lax.dot_general(_to16(wvt_ref[r0 // 2:r1 // 2, :]), hval(w, 1), NT,
                                              preferred_element_type=f32))

        def shifted(w, off):
            for n in range(off // 128, off // 128 + 5):
                chk("r", w, n)
                chk("b", 9, n)
            return raw_ref[_t(w), off:off + D] + _rows(bias_ref[16:24, off:off + D], 128)

        def qfin(w):
            qstore(w, 1, shifted(w, 0))

        def kfin(w):
            kstore(w, 1, shifted(w, D))

        def sel(m, a, b):
            if a is None and b is None:
                return None
            return jnp.where(m, neg32 if a is None else a, neg32 if b is None else b)

        def qparts(w, g):
            start, a = (80 * g) % 128, (80 * g) // 128
            chk("q", w)
            for ww in range(max(w - 2, 0), w + 1):
                chk("k", ww)
            hm = [_circ_mask(lane32, start + DH * i, DH) for i in range(4)]
            qs = []
            for j in range(4):
                r = slice(128 * w + 32 * j, 128 * w + 32 * j + 32)
                qj = q_ref[r, _t(a)]
                if start + 80 > 128:
                    qj = jnp.where(lane32 >= start, qj, q_ref[r, _t(a + 1)])
                qs.append(qj)
            return hm, qs

        def edge_scores(w, g, half=None):
            hm, qs = qparts(w, g)
            t2 = 64 * w
            t0 = t2 - 128
            u = [None] * 4
            for j in (3, 2, 1, 0):
                qm = jnp.concatenate([jnp.where(hm[(j - c) % 4], qs[j], 0.0) for c in range(4)],
                                     axis=0)
                kw = k_ref[t2:t2 + 16 * (j + 1), _t(g)]
                if w >= 2:
                    kw = jnp.concatenate([kw, k_ref[t0 + 16 * j:t0 + 64, _t(g)]], axis=0)
                if half is not None:
                    kw = kw[40 * half:40 * half + 40]
                s = lax.dot_general(_to16(kw), qm.astype(bf16), NT, preferred_element_type=f32)
                if half == 0:
                    st["e", j] = s
                    continue
                if half == 1:
                    s = jnp.concatenate([st.pop(("e", j)), s], axis=0)
                blk = [s[32 * r:32 * r + 32] for r in range(s.shape[0] // 32)]
                if w >= 2:
                    u[j] = blk[:j] + [jnp.where(mask_up, blk[j + 1], blk[j])] + blk[j + 2:]
                else:
                    u[j] = blk[:j] + [jnp.where(mask_up, NEG, blk[j])] + [None] * (3 - j)
            if half == 0:
                return
            e = [[], [], [], []]
            for r in range(4):
                t = [sel(bit0, u[j][r], u[(j + 1) % 4][r]) for j in range(4)]
                for i in range(4):
                    e[i].append(sel(bit1, t[i], t[(i + 2) % 4]))
            ms = []
            for i in range(4):
                se = jnp.concatenate(e[i], axis=0)
                ms.append(_colmax8([se]))
                s_ref[g % 4, i, 0:128, :] = se
            st["m", w, g] = ms

        def a_edge(w, g):
            if w >= 2:
                edge_scores(w, g)
            elif g % 2 == 0:
                edge_scores(w, g)
                edge_scores(w, g + 1)

        def a_mid(w, g):
            ms = st["m", w, g]
            if w >= 1:
                hm, qs = qparts(w, g)
                qm = jnp.concatenate([jnp.where(hm[i], qs[(i + c) % 4], 0.0)
                                      for i in range(4) for c in range(4)], axis=0)
                t1 = 64 * (w - 1)
                smid = lax.dot_general(_to16(k_ref[t1:t1 + 64, _t(g)]), qm.astype(bf16),
                                       NT, preferred_element_type=f32)
                for i in range(4):
                    sm = smid[:, _t(i)]
                    ms[i] = _colmax8([ms[i], sm])
                    s_ref[g % 4, i, 128:256, :] = sm
            st["m", w, g] = [jnp.max(m8, axis=0, keepdims=True) for m8 in ms]

        def pv(w, g, kt, ps):
            res = st.setdefault(("r", w, g), [None] * 4)
            for v in range(10 * g, 10 * g + 10):
                chk("v", w - 2 + kt, v)
            for i, p in enumerate(ps):
                hd = 4 * g + i
                d = jnp.dot(vt_ref[24 * hd:24 * hd + 24, _t(w - 2 + kt)], p.astype(bf16),
                            preferred_element_type=f32)
                res[i] = d if res[i] is None else d + res[i]

        def c_mid(w, g):
            if w >= 1:
                pv(w, g, 1, [jnp.exp2(s_ref[g % 4, i, 128:256, :] - m)
                             for i, m in enumerate(st["m", w, g])])

        def c_old(w, g):
            pe = [jnp.exp2(s_ref[g % 4, i, 0:128, :] - m) for i, m in enumerate(st.pop(("m", w, g)))]
            if w >= 2:
                up = [row128 > ((lane128 + 32 * i) & 127) for i in range(4)]
                pv(w, g, 0, [jnp.where(up[i], pe[i], 0.0) for i in range(4)])
                pe = [jnp.where(up[i], 0.0, pe[i]) for i in range(4)]
            st["p", w, g] = pe

        def c_new(w, g):
            pv(w, g, 2, st.pop(("p", w, g)))
            res = st.pop(("r", w, g))
            res = [r if i == 0 else pltpu.roll(r, 32 * i, 1) for i, r in enumerate(res)]
            out = []
            for e in (0, 2):
                re, ro = res[e], res[e + 1]
                inv = 1.0 / jnp.where(sub8, ro[0:8], re[16:24])
                swp = pltpu.roll(inv, 4, 0)
                ie = jnp.where(sub8, swp, inv)
                io = jnp.where(sub8, inv, swp)
                out += [re[0:8] * ie, re[8:16] * ie,
                        jnp.where(sub8, re[16:24], ro[0:8]) * swp,
                        ro[8:16] * io, ro[16:24] * io]
            ot_ref[w, 80 * g:80 * g + 80, :] = jnp.concatenate(out, axis=0)
            have.add(("t", w, g))

        def ostore(w):
            for g in range(NG):
                chk("t", w, g)
            a_ref[_t(w), :] = ot_ref[w].T
            have.add(("a", w))

        def slide():
            k_ref[0:W // 2, :] = k_ref[W // 2:W, :]
            vt_ref[:, 0:W] = vt_ref[:, W:2 * W]

        def ln2(b):
            h2 = _ln(x1_ref[_t(b), :]) * modv(4) + modv(3)
            st["yf", b] = _ln(h2)
            st["y", b] = st["yf", b].astype(bf16)

        def oproj(b, n0, n1, nb=1):
            assert (n0, n1) == (0, 5)
            m = 128 * nb
            o = a_ref[W + 128 * b:W + 128 * b + m, :].astype(bf16)
            attn = jnp.dot(o, _to16(wo(0, D)), preferred_element_type=f32)
            ga = mod(2 * D, 3 * D, m)
            x1_ref[128 * b:128 * b + m, :] = (
                x_ref[rows(bblk, 128 * b, m), :].astype(f32) + ga * attn)
            for i in range(b, b + nb):
                ln2(i)

        def ofin(b):
            for n in range(5):
                chk("x", b, n)
            x1_ref[_t(b), :] = (x_ref[rows(bblk, 128 * b, 128), :].astype(f32)
                                + modv(2) * x1_ref[_t(b), :])
            ln2(b)

        def act(b, lo, hi, h1):
            st.setdefault(("g1", b), []).append(_gelu(h1 + _rows(bias_ref[0:8, lo:hi], 128)))

        def mlp1(b, n0, n1):
            lo, hi = 128 * n0, 128 * n1
            act(b, lo, hi, lax.dot_general(st["y", b], _to16(w1t(lo, hi)), NT,
                                           preferred_element_type=f32))

        def mlp1_tail(_, n0, n1):
            wt = _to16(w1t(FM, F))
            for b in range(n0, n1):
                st["tt", b] = lax.dot_general(wt, st["y", b], NT, preferred_element_type=f32)
            if n1 == 2:
                h1 = jnp.concatenate([st["tt", 0], st["tt", 1]], axis=0).T
                st["gt"] = _gelu(h1 + _rows(bias_ref[0:8, FM:FM + 128], 128))

        def mlp2(b, n0, n1, split=1):
            lo, hi = 128 * n0, 128 * n1
            if isinstance(st["g1", b], list):
                assert sum(g.shape[1] for g in st["g1", b]) == FM
                tail = st["gt"][:, 0:64] if b == 0 else jnp.where(lane128 >= 64, st["gt"], 0.0)
                st["g1", b] = jnp.concatenate(st["g1", b] + [tail], axis=1)
            wd = w2(lo, hi)
            if b == 1:
                wd = jnp.concatenate([wd[0:FM // 2], wd[F // 2 - 64:F // 2]], axis=0)
            m = 128 // split
            for k in range(split):
                g1 = memo(("g", b, split, k), lambda: st["g1", b][m * k:m * k + m].astype(bf16))
                out = jnp.dot(g1, _to16(wd), preferred_element_type=f32)
                out = out + _rows(bias_ref[8:16, lo:hi], m)
                gb = mod(5 * D + lo, 5 * D + hi, m)
                r0 = 128 * b + m * k
                o_ref[rows(bblk, r0, m, m), lo:hi] = (
                    x1_ref[r0:r0 + m, lo:hi] + gb * out).astype(o_ref.dtype)
            if mode == "last" and n1 >= 3:
                done = st.get(("wb", b), 0)
                r = rows(bblk, 128 * b, 128)
                pltpu.make_async_copy(o_ref.at[r, 128 * done:hi], o_hbm.at[r, 128 * done:hi],
                                      osem).start()
                st["wb", b] = n1

        def tiles(n0, n1, lhs, rhs, fin, dims=NN):
            for n in range(n0, n1):
                acc = None
                for k in range(5):
                    d = lax.dot_general(lhs(n, k), rhs(n, k), dims, preferred_element_type=f32)
                    acc = d if acc is None else d + acc
                    if k == 4:
                        fin(n, acc)
                    yield

        def ptile(k):
            return slice(64 * k, 64 * k + 64)

        def wqk_tile(n, k):
            assert (wqk_name(128 * n), 128 * n) in st
            return _to16(wqk_ref[ptile(k), _t(n)])

        def gen_m(_, n0, n1):
            def rhs(n, k):
                chk("w", "sa" if n < 5 else "mb" if n < 25 else "gb")
                return wmod_in[_t(k), _t(n)]
            return tiles(n0, n1, lambda n, k: st["sc"][:, _t(k)], rhs,
                         lambda n, acc: mod_store(128 * n, acc))

        def gen_b(_, n0, n1):
            def fin(n, acc):
                bias_ref[16:24, _t(n)] = acc
                have.add(("b", 9, n))
            return tiles(n0, n1, lambda n, k: mod(128 * k, 128 * k + 128, 8), wqk_tile, fin)

        def gen_raw(off, w, n0, n1):
            def fin(n, acc):
                raw_ref[_t(w), _t(n)] = acc
                have.add(("r", w, n))
            return tiles(
                off + n0, off + n1, lambda n, k: st["hs", w, k],
                lambda n, k: _to16(memo(("qw", w, n), lambda: wqk(128 * n, 128 * n + 128))[ptile(k)]),
                fin)

        def gen_v(w, n0, n1):
            def lhs(n, k):
                chk("w", "v")
                return _to16(wvt_ref[ptile(n), _t(k)])
            return tiles(n0, n1, lhs, lambda n, k: htile(w, k),
                         lambda n, acc: vstore(w, 128 * n, 128 * n + 128, acc), NT)

        def gen_o(b, n0, n1):
            def lhs(n, k):
                chk("a", b)
                return memo(("ot", b, k), lambda: a_ref[_t(b), _t(k)].astype(bf16))

            def fin(n, acc):
                x1_ref[_t(b), _t(n)] = acc
                have.add(("x", b, n))
            return tiles(
                n0, n1, lhs,
                lambda n, k: _to16(memo(("ow", b, n), lambda: wo(128 * n, 128 * n + 128))[ptile(k)]),
                fin)

        def gen_u(b, n0, n1):
            return tiles(
                n0, n1,
                lambda n, k: memo(("yt", b, k), lambda: st["yf", b][:, _t(k)].astype(bf16)),
                lambda n, k: _to16(memo(("uw", b, n), lambda: w1t(128 * n, 128 * n + 128))[:, _t(k)]),
                lambda n, acc: act(b, 128 * n, 128 * n + 128, acc), NT)

        matmuls = dict(v=vproj, Q=qproj2, K=kproj2, o=oproj, O=P(oproj, nb=2),
                       u=mlp1, t=mlp1_tail, d=mlp2, D=P(mlp2, split=2))
        gens = dict(m=gen_m, b=gen_b, j=P(gen_raw, 0), i=P(gen_raw, 5), v=gen_v, o=gen_o, u=gen_u)
        stages = dict(l=ln1, c=hscale, q=qfin, k=kfin, s=ostore, f=ofin)
        cursor = {("m", 0): 10, ("b", 1): 5}
        queues = dict(L=iter(()), s=iter(()))

        def advance(tok):
            kind, blk, cnt = tok[0], int(tok[1]), int(tok[3:])
            n0 = cursor.get((kind.lower(), blk), 0)
            cursor[kind.lower(), blk] = n0 + cnt
            return kind, blk, n0, n0 + cnt

        def emit(spec):
            for tok in spec.split():
                if tok[0] == "+":
                    for name in tok[1:].split(","):
                        cps[name]().start()
                        flying.add(name)
                elif tok[0] == "?":
                    wait(tok[1:].split(","))
                elif tok[0] == "!":
                    stages[tok[1]](int(tok[2]))
                elif tok[0] == "@":
                    kind, *args = advance(tok[1:])
                    qn = "s" if kind in "mb" else "L"
                    queues[qn] = itertools.chain(queues[qn], gens[kind](*args))
                elif tok[0] == "#":
                    for qn in tok[1:]:
                        for _ in range(4):
                            next(queues[qn], None)
                else:
                    kind, *args = advance(tok)
                    matmuls[kind](*args)

        def attention(ws, fills):
            groups = [(w, g) for w in ws for g in range(NG)]
            for g in groups[:LEAD]:
                a_edge(*g)
                a_mid(*g)
            for n, g in enumerate(groups):
                emit(fills[n])
                ahead = groups[n + LEAD] if n + LEAD < len(groups) else None
                split = first and ahead and ahead[0] >= 2 and "L" not in fills[n]
                if split:
                    edge_scores(*ahead, half=0)
                c_mid(*g)
                if split:
                    edge_scores(*ahead, half=1)
                elif ahead:
                    a_edge(*ahead)
                c_old(*g)
                if ahead:
                    a_mid(*ahead)
                c_new(*g)
            slide()

        if first:
            emit(FIRST_PRE)
            attention(range(4), FIRST_FILL.split("|"))
            emit(FIRST_POST)
            assert next(queues["L"], 1) and next(queues["s"], 1) and not flying
        elif mode == "steady":
            emit(STEADY_PRE)
            attention((2, 3), STEADY_FILL.split("|"))
            emit(STEADY_POST)
        else:
            emit(LAST)
            pltpu.make_async_copy(o_ref, o_hbm, osem).wait()

    pl.when(step == 0)(P(body, "first"))
    pl.when(jnp.logical_and(step > 0, step < NB - 1))(P(body, "steady"))
    pl.when(step == NB - 1)(P(body, "last"))


@jax.jit
def pallas_adaLN_cond__sliding_block__mixer_channel_mlp__prompt_kernel(
    A_x: jax.Array,
    A_wqkv: jax.Array,
    A_wo: jax.Array,
    B_x: jax.Array,
    B_w1: jax.Array,
    B_b1: jax.Array,
    B_w2: jax.Array,
    B_b2: jax.Array,
    c: jax.Array,
    w_mod: jax.Array,
):
    del B_x
    hbm = pl.BlockSpec(memory_space=pl.ANY)
    out = pl.pallas_call(
        _kernel,
        grid=(NB,),
        in_specs=[hbm] * 9,
        out_specs=hbm,
        out_shape=jax.ShapeDtypeStruct((S, D), A_x.dtype),
        scratch_shapes=[
            pltpu.VMEM((S, D), bf16),
            pltpu.VMEM((S, D), bf16),
            pltpu.VMEM((D, 3 * D), bf16),
            pltpu.VMEM((D, D), bf16),
            pltpu.VMEM((F, D), bf16),
            pltpu.VMEM((F, D), bf16),
            pltpu.VMEM((D, 6 * D), bf16),
            pltpu.VMEM((F,), bf16),
            pltpu.VMEM((D,), bf16),
            pltpu.VMEM((1, D), bf16),
            pltpu.VMEM((D // 2, 2 * D), u32),
            pltpu.VMEM((D // 2, D), u32),
            pltpu.VMEM((F // 2, D), u32),
            pltpu.VMEM((F // 2, D), u32),
            pltpu.SemaphoreType.DMA((4,)),
            pltpu.VMEM((8, 6 * D), f32),
            pltpu.VMEM((24, 1792), f32),
            pltpu.VMEM((D // 2, D), u32),
            pltpu.VMEM((2 * W, D), f32),
            pltpu.VMEM((W, NG * 128), u32),
            pltpu.VMEM((24 * H, 2 * W), f32),
            pltpu.VMEM((2 * W, D), f32),
            pltpu.VMEM((4, 4, 256, 128), f32),
            pltpu.VMEM((4, D, 128), f32),
            pltpu.VMEM((TQ, D), f32),
            pltpu.VMEM((2 * W, D), f32),
            pltpu.VMEM((2 * W, 2 * D), f32),
        ],
        compiler_params=pltpu.CompilerParams(
            dimension_semantics=("arbitrary",),
            vmem_limit_bytes=100 * 1024 * 1024),
        name="fused_block",
    )(A_x.reshape(S, D), A_wqkv, A_wo, B_w1.T, B_b1, B_w2, B_b2, c, w_mod)
    return out.reshape(1, S, D)
```
